```python
import os as _os
_os.environ.setdefault("JAX_PLATFORMS", "cpu")
import jax
import jax.numpy as jnp

def _softmax(x, axis=-1):
    return jax.nn.softmax(x, axis=axis)
def _gelu(x):
    return jax.nn.gelu(x, approximate=True)
def _silu(x):
    return jax.nn.silu(x)
def _sigmoid(x):
    return jax.nn.sigmoid(x)
def _layernorm(x, axis=-1, eps=1e-5):
    m = jnp.mean(x, axis=axis, keepdims=True)
    v = jnp.var(x, axis=axis, keepdims=True)
    return (x - m) / jnp.sqrt(v + eps)
def _scatter_add(tgt, idx, src, axis=0):
    return tgt.at[idx].add(src)
def _segment_sum(src, seg, n):
    return jax.ops.segment_sum(src, seg, n)
class _Rng:
    def __init__(self, key):
        self._k = key
    def _next(self):
        self._k, sub = jax.random.split(self._k)
        return sub
    def normal(self, shape):
        return jax.random.normal(self._next(), shape, dtype=jnp.bfloat16)
    def randint(self, lo, hi, shape):
        return jax.random.randint(self._next(), shape, lo, hi, dtype=jnp.int32)
    def uniform(self, shape, lo=0.0, hi=1.0):
        return jax.random.uniform(self._next(), shape, jnp.bfloat16, lo, hi)
    def permutation(self, n):
        return jax.random.permutation(self._next(), n)


kernel_name = 'interleave_layers__gqa_block_cached__dense_activation_mish__decode'

def setup_inputs():
    _rng = _Rng(jax.random.key(int.from_bytes(__import__("os").urandom(4), "little")))
    _w = (lambda a: (lambda t: t.astype(jnp.bfloat16) if jnp.issubdtype(t.dtype, jnp.floating) else t)(jnp.asarray(a)))
    def _A_setup():
        B, Sq, D = 1, 1, 512
        Hq, Hkv, Sk, Dh = 32, 8, 65536, 128
        assert Hq % Hkv == 0, (Hq, Hkv)
        return {
            "x": _w((lambda *s: _rng.normal(s) * 0.05)(B, Sq, D)),
            "k_cache": _w((lambda *s: _rng.normal(s) * 1.6)(B, Hkv, Sk, Dh)),
            "v_cache": _w((lambda *s: _rng.normal(s) * 1.6)(B, Hkv, Sk, Dh)),
            "wq": _w((lambda *s: _rng.normal(s) * 1.6)(D, Hq * Dh) * (D ** -0.5)),
            "wo": _w((lambda *s: _rng.normal(s) * 1.6)(Hq * Dh, D) * ((Hq * Dh) ** -0.5)),
        }
    _A_in = _A_setup()

    def _B_setup():
        B, S, D, F = 1, 1, 512, 1792
        return {
            "x": _w((lambda *s: _rng.normal(s) * 0.05)(B, S, D)),
            "w1": _w((lambda *s: _rng.normal(s) * 0.8)(D, F) * (D ** -0.5)),
            "b1": _w((lambda *s: _rng.normal(s) * 0.8)(F)),
            "w2": _w((lambda *s: _rng.normal(s) * 0.8)(F, D) * (F ** -0.5)),
        }
    _B_in = _B_setup()

    return {
        "A_x": _A_in["x"],
        "A_k_cache": _A_in["k_cache"],
        "A_v_cache": _A_in["v_cache"],
        "A_wq": _A_in["wq"],
        "A_wo": _A_in["wo"],
        "B_x": _B_in["x"],
        "B_w1": _B_in["w1"],
        "B_b1": _B_in["b1"],
        "B_w2": _B_in["w2"],
    }

def reference(A_x, A_k_cache, A_v_cache, A_wq, A_wo, B_x, B_w1, B_b1, B_w2):
    def _A_ref(x, k_cache, v_cache, wq, wo):
        B, Sq, D = x.shape
        Hq, Dh = 32, 128
        Hkv = k_cache.shape[1]
        rep = Hq // Hkv
        q = (lambda x, *d: x.transpose(*d))((x @ wq).reshape(B, Sq, Hq, Dh), 0, 2, 1, 3)
        k = jnp.repeat(k_cache, rep, axis=1)
        v = jnp.repeat(v_cache, rep, axis=1)
        scores = jnp.einsum("bhqd,bhkd->bhqk", q, k) * (Dh ** -0.5)
        p = _softmax(scores, axis=-1)
        o = jnp.einsum("bhqk,bhkd->bhqd", p, v)
        return (lambda x, *d: x.transpose(*d))(o, 0, 2, 1, 3).reshape(B, Sq, Hq * Dh) @ wo

    def _B_ref(x, w1, b1, w2):
        h = jnp.einsum("bsd,df->bsf", x, w1) + b1
        sp = jnp.log1p(jnp.exp(-jnp.abs(h))) + jnp.where(h > 0, h, jnp.zeros_like(h))
        act = h * jnp.tanh(sp)
        return jnp.einsum("bsf,fd->bsd", act, w2)

    x = A_x
    x = x + _A_ref(_layernorm(x, axis=-1), A_k_cache, A_v_cache, A_wq, A_wo)
    x = x + _B_ref(_layernorm(x, axis=-1), B_w1, B_b1, B_w2)
    x = x + _A_ref(_layernorm(x, axis=-1), A_k_cache, A_v_cache, A_wq, A_wo)
    x = x + _B_ref(_layernorm(x, axis=-1), B_w1, B_b1, B_w2)
    return x
```

```python
import jax
import jax.numpy as jnp
from jax import lax
import jax.experimental.pallas as pl
import jax.experimental.pallas.tpu as pltpu

_D = 512
_HQ = 32
_DH = 128
_EPS = 1e-5
_NT = (((1,), (1,)), ((), ()))


def _layernorm(x):
    m = jnp.mean(x, axis=-1, keepdims=True)
    c = x - m
    v = jnp.mean(c * c, axis=-1, keepdims=True)
    return c / jnp.sqrt(v + _EPS)


def build(hkv, sk, f_dim, BS, S, D1, D2, prio=(0, 0)):
    rep = _HQ // hkv
    uph = sk // BS
    U = hkv * uph
    M = U - S

    def kernel(x_hbm, k_hbm, v_hbm, wq_hbm, wo_hbm, w1_hbm, b1_hbm, w2_hbm, out_ref,
               kbuf, vbuf, wq, wo, w1, w2, b1, xs, q_ref, m_ref, l_ref, acc_ref,
               ksem, vsem, wsem):

        def kv_copies(unit, slot):
            rows = pl.ds(pl.multiple_of(unit * BS, BS), BS)
            return (pltpu.make_async_copy(k_hbm.at[rows], kbuf.at[slot], ksem.at[slot]),
                    pltpu.make_async_copy(v_hbm.at[rows], vbuf.at[slot], vsem.at[slot]))

        def issue(unit, slot):
            kc, vc = kv_copies(unit, slot)
            kc.start(priority=prio[0])
            vc.start(priority=prio[1])

        def wait(slot):
            kc, vc = kv_copies(0, slot)
            kc.wait()
            vc.wait()

        def process(slot, g):
            q = q_ref[g].astype(jnp.bfloat16)
            s = lax.dot_general(q, kbuf[slot], _NT, preferred_element_type=jnp.float32)
            m_old = m_ref[g]
            m_new = jnp.maximum(m_old, jnp.max(s, axis=-1, keepdims=True))
            alpha = jnp.exp(m_old - m_new)
            p = jnp.exp(s - m_new[:, :1])
            l_ref[g] = alpha * l_ref[g] + jnp.sum(p, axis=-1, keepdims=True)
            m_ref[g] = m_new
            pv = jnp.dot(p.astype(jnp.bfloat16), vbuf[slot], preferred_element_type=jnp.float32)
            acc_ref[g] = alpha * acc_ref[g] + pv

        row128 = lax.broadcasted_iota(jnp.int32, (8, _DH), 0)

        def q_proj(x):
            xn = _layernorm(x).astype(jnp.bfloat16)
            for g in range(hkv):
                qf = jnp.dot(xn, wq[:, g * rep * _DH:(g + 1) * rep * _DH],
                             preferred_element_type=jnp.float32)
                qg = jnp.zeros((8, _DH), jnp.float32)
                for hh in range(rep):
                    qg = jnp.where(row128 == hh, qf[:, hh * _DH:(hh + 1) * _DH], qg)
                q_ref[g] = qg * (_DH ** -0.5)
            m_ref[...] = jnp.full(m_ref.shape, -jnp.inf, jnp.float32)
            l_ref[...] = jnp.zeros(l_ref.shape, jnp.float32)
            acc_ref[...] = jnp.zeros(acc_ref.shape, jnp.float32)

        def o_proj(x):
            out = x
            for g in range(hkv):
                og = (acc_ref[g] / l_ref[g]).astype(jnp.bfloat16)
                flat = jnp.concatenate(
                    [jnp.broadcast_to(og[hh:hh + 1, :], (8, _DH)) for hh in range(rep)], axis=1)
                out = out + jnp.dot(flat, wo[g * rep * _DH:(g + 1) * rep * _DH, :],
                                    preferred_element_type=jnp.float32)
            return out

        def mlp_up(x):
            xn = _layernorm(x).astype(jnp.bfloat16)
            h = jnp.dot(xn, w1[...], preferred_element_type=jnp.float32) + b1[...].astype(jnp.float32).reshape(1, f_dim)
            sp = jnp.log1p(jnp.exp(-jnp.abs(h))) + jnp.where(h > 0, h, 0.0)
            return (h * jnp.tanh(sp)).astype(jnp.bfloat16)

        def mlp_down(x, act):
            return x + jnp.dot(act, w2[...], preferred_element_type=jnp.float32)

        c_x = pltpu.make_async_copy(x_hbm, xs, wsem.at[0])
        c_wq = pltpu.make_async_copy(wq_hbm, wq, wsem.at[1])
        c_wo = pltpu.make_async_copy(wo_hbm, wo, wsem.at[2])
        c_w1 = pltpu.make_async_copy(w1_hbm, w1, wsem.at[3])
        c_b1 = pltpu.make_async_copy(b1_hbm, b1, wsem.at[4])
        c_w2 = pltpu.make_async_copy(w2_hbm, w2, wsem.at[5])

        c_x.start()
        c_wq.start()
        for u in range(D1):
            issue(u, u % S)
        c_wo.start()
        c_x.wait()
        c_wq.wait()
        x0 = jnp.broadcast_to(xs[...].astype(jnp.float32), (8, _D))
        q_proj(x0)

        def body1(u, c):
            @pl.when(u + D1 < U)
            def _():
                issue(u + D1, (u + D1) % S)

            @pl.when(u == U - D1)
            def _():
                c_b1.start()
                c_w1.start()
                c_w2.start()

            slot = u % S
            wait(slot)
            process(slot, u // uph)
            return c
        lax.fori_loop(0, U, body1, 0)

        c_wo.wait()
        x1 = o_proj(x0)
        c_b1.wait()
        c_w1.wait()
        act = mlp_up(x1)
        c_w2.wait()
        x2 = mlp_down(x1, act)
        q_proj(x2)

        for r in range(D2):
            process((M + r) % S, (M + r) // uph)
            issue(r, (M + r) % S)

        def body2(j, c):
            r = j + D2

            @pl.when(r < S)
            def _():
                process((M + r) % S, (M + r) // uph)

            @pl.when(r < M)
            def _():
                issue(r, (M + r) % S)

            slot = (M + j) % S
            wait(slot)
            process(slot, j // uph)
            return c
        lax.fori_loop(0, M, body2, 0)
        if S > M + D2:
            def body3(r, c):
                process((M + r) % S, (M + r) // uph)
                return c
            lax.fori_loop(M + D2, S, body3, 0)

        x3 = o_proj(x2)
        act = mlp_up(x3)
        x4 = mlp_down(x3, act)
        out_ref[...] = x4[:1, :].astype(out_ref.dtype)

    return pl.pallas_call(
        kernel,
        out_shape=jax.ShapeDtypeStruct((1, _D), jnp.bfloat16),
        in_specs=[pl.BlockSpec(memory_space=pl.ANY)] * 8,
        out_specs=pl.BlockSpec(memory_space=pltpu.VMEM),
        scratch_shapes=[
            pltpu.VMEM((S, BS, _DH), jnp.bfloat16),
            pltpu.VMEM((S, BS, _DH), jnp.bfloat16),
            pltpu.VMEM((_D, _HQ * _DH), jnp.bfloat16),
            pltpu.VMEM((_HQ * _DH, _D), jnp.bfloat16),
            pltpu.VMEM((_D, f_dim), jnp.bfloat16),
            pltpu.VMEM((f_dim, _D), jnp.bfloat16),
            pltpu.VMEM((f_dim,), jnp.bfloat16),
            pltpu.VMEM((1, _D), jnp.bfloat16),
            pltpu.VMEM((hkv, 8, _DH), jnp.float32),
            pltpu.VMEM((hkv, 8, _DH), jnp.float32),
            pltpu.VMEM((hkv, 8, _DH), jnp.float32),
            pltpu.VMEM((hkv, 8, _DH), jnp.float32),
            pltpu.SemaphoreType.DMA((S,)),
            pltpu.SemaphoreType.DMA((S,)),
            pltpu.SemaphoreType.DMA((6,)),
        ],
        compiler_params=pltpu.CompilerParams(vmem_limit_bytes=128 * 1024 * 1024),
    )


@jax.jit
def pallas_interleave_layers__gqa_block_cached__dense_activation_mish__decode_kernel(
    A_x: jax.Array,
    A_k_cache: jax.Array,
    A_v_cache: jax.Array,
    A_wq: jax.Array,
    A_wo: jax.Array,
    B_x: jax.Array,
    B_w1: jax.Array,
    B_b1: jax.Array,
    B_w2: jax.Array,
):
    del B_x
    _, hkv, sk, dh = A_k_cache.shape
    f_dim = B_w1.shape[1]
    out = build(hkv, sk, f_dim, 4096, 58, 4, 4)(
        A_x.reshape(1, _D),
        A_k_cache.reshape(hkv * sk, dh),
        A_v_cache.reshape(hkv * sk, dh),
        A_wq, A_wo, B_w1, B_b1, B_w2)
    return out.reshape(1, 1, _D)
```

```python
import functools

import jax
import jax.numpy as jnp
import numpy as np
from jax import lax
import jax.experimental.pallas as pl
import jax.experimental.pallas.tpu as pltpu

_D = 512
_HQ = 32
_DH = 128
_EPS = 1e-5
_NT = (((1,), (1,)), ((), ()))
_I32 = jnp.int32


def _c32(x):
    return np.int32(np.uint32(x))


def _srl(x, n):
    return lax.shift_right_logical(x, np.int32(n))


def _layernorm(x):
    m = jnp.mean(x, axis=-1, keepdims=True)
    c = x - m
    v = jnp.mean(c * c, axis=-1, keepdims=True)
    return c / jnp.sqrt(v + _EPS)


def build(hkv, sk, f_dim, T, R, NC, pieces, force_bad=None, nobounds=False, split_w=True, lead_units=1):
    lead = lead_units * NC
    BS = T * 128
    rep = _HQ // hkv
    uph = sk // BS
    U = hkv * uph
    M = U - R - NC
    NSM = (T + 1) // 2
    NE = (T + 2) // 3

    def kernel(x_hbm, k_hbm, v_hbm, wq_hbm, wo_hbm, w1_hbm, b1_hbm, w2_hbm, out_ref,
               kbuf, vbuf, ksm, kex, vsm, vex, wq, wo, w1, w2, b1, xs,
               q_ref, m_ref, l_ref, acc_ref, base_ref, ok_ref, redo_ref,
               ksem, vsem, wsem):

        def issue(unit, slot):
            base = pl.multiple_of(unit * BS, BS)
            off = 0
            for n in pieces:
                rows = pl.ds(base + off, n)
                dst = pl.ds(off, n)
                pltpu.make_async_copy(k_hbm.at[rows], kbuf.at[slot, dst], ksem.at[slot]).start(priority=0)
                pltpu.make_async_copy(v_hbm.at[rows], vbuf.at[slot, dst], vsem.at[slot]).start(priority=1)
                off += n
            assert off == BS

        def wait(slot):
            pltpu.make_async_copy(k_hbm.at[pl.ds(0, BS)], kbuf.at[slot], ksem.at[slot]).wait()
            pltpu.make_async_copy(v_hbm.at[pl.ds(0, BS)], vbuf.at[slot], vsem.at[slot]).wait()

        def attend(g, get_k, get_v):
            q = q_ref[g].astype(jnp.bfloat16)
            ss = [lax.dot_general(q, get_k(t), _NT, preferred_element_type=jnp.float32)
                  for t in range(T)]
            mx = jnp.max(functools.reduce(jnp.maximum, ss), axis=-1, keepdims=True)
            m_old = m_ref[g]
            m_new = jnp.maximum(m_old, mx)
            alpha = jnp.exp(m_old - m_new)
            ps = [jnp.exp(s - m_new) for s in ss]
            l_ref[g] = alpha * l_ref[g] + functools.reduce(jnp.add, ps)
            m_ref[g] = m_new
            acc = alpha * acc_ref[g]
            for t in range(T):
                acc = acc + jnp.dot(ps[t].astype(jnp.bfloat16), get_v(t),
                                    preferred_element_type=jnp.float32)
            acc_ref[g] = acc

        def raw_tile(buf, slot):
            return lambda t: buf[slot, t * 128:(t + 1) * 128, :]

        def process_raw(slot, g):
            attend(g, raw_tile(kbuf, slot), raw_tile(vbuf, slot))

        def encoder(buf, slot, sm_ref, ex_ref, c, which):
            st = {}
            t0 = buf[slot, 0:128, :]
            amax = jnp.max(jnp.abs(t0.astype(jnp.float32)), axis=(0, 1), keepdims=True)
            emax = _srl(pltpu.bitcast(jnp.broadcast_to(amax, (8, 128)), _I32), 23) & 0xFF
            base = jnp.clip(emax - 29, 0, 224)
            basep = (base << 7) | (base << 23)
            base_ref[2 * c + which] = jnp.max(basep)
            basep = jnp.broadcast_to(basep[:1, :], (64, 128))
            st["bad"] = jnp.zeros((8, 128), _I32)

            def get(t):
                tile = buf[slot, t * 128:(t + 1) * 128, :]
                w = pltpu.bitcast(tile, _I32)
                d = (w & _c32(0x7F807F80)) - basep
                st["bad"] = functools.reduce(
                    jnp.bitwise_or, [d[8 * i:8 * i + 8, :] for i in range(8)], st["bad"])
                j = t % 3
                if j == 0:
                    st["e"] = _srl(d, 7)
                elif j == 1:
                    st["e"] = st["e"] | _srl(d, 2)
                else:
                    st["e"] = st["e"] | (d << 3)
                if j == 2 or t == T - 1:
                    ex_ref[c, (t // 3) * 64:(t // 3 + 1) * 64, :] = st["e"]
                if t % 2 == 0:
                    st["s"] = (w & _c32(0x007F007F)) | (_srl(w, 8) & _c32(0x00800080))
                else:
                    st["s"] = st["s"] | ((w & _c32(0x007F007F)) << 8) | (w & _c32(0x80008000))
                if t % 2 == 1 or t == T - 1:
                    sm_ref[c, (t // 2) * 64:(t // 2 + 1) * 64, :] = st["s"]
                return tile

            def fin():
                return st["bad"] & _c32(0xF000F000)
            return get, fin

        def process_encode(slot, g, c):
            gk, fk = encoder(kbuf, slot, ksm, kex, c, 0)
            gv, fv = encoder(vbuf, slot, vsm, vex, c, 1)
            attend(g, gk, gv)
            bad = fk() | fv()
            anybad = jnp.max(jnp.where(bad != 0, 1.0, 0.0))
            ok = anybad == 0.0
            if force_bad is not None:
                ok = jnp.logical_and(ok, (c % force_bad) != 1)
            ok_ref[c] = ok.astype(_I32)
            n = redo_ref[U]

            @pl.when(jnp.logical_not(ok))
            def _():
                redo_ref[n] = M + c
                redo_ref[U] = n + 1

        def decoder(sm_ref, ex_ref, c, which):
            basep = base_ref[2 * c + which]

            def get(t):
                sm = sm_ref[c, (t // 2) * 64:(t // 2 + 1) * 64, :]
                e = ex_ref[c, (t // 3) * 64:(t // 3 + 1) * 64, :]
                j = t % 3
                if j == 0:
                    ef = (e << 7) & _c32(0x0F800F80)
                elif j == 1:
                    ef = (e << 2) & _c32(0x0F800F80)
                else:
                    ef = _srl(e, 3) & _c32(0x0F800F80)
                if t % 2 == 0:
                    a = sm & _c32(0x00FF00FF)
                    a = (a | (a << 8)) & _c32(0x807F807F)
                else:
                    a = sm & _c32(0xFF00FF00)
                    a = (a | _srl(a, 8)) & _c32(0x807F807F)
                return pltpu.bitcast((a | ef) + basep, jnp.bfloat16)
            return get

        def process_packed(c):
            attend((M + c) // uph, decoder(ksm, kex, c, 0), decoder(vsm, vex, c, 1))

        row128 = lax.broadcasted_iota(_I32, (8, _DH), 0)

        def q_proj(x):
            xn = _layernorm(x).astype(jnp.bfloat16)
            for g in range(hkv):
                qf = jnp.dot(xn, wq[:, g * rep * _DH:(g + 1) * rep * _DH],
                             preferred_element_type=jnp.float32)
                qg = jnp.zeros((8, _DH), jnp.float32)
                for hh in range(rep):
                    qg = jnp.where(row128 == hh, qf[:, hh * _DH:(hh + 1) * _DH], qg)
                q_ref[g] = qg * (_DH ** -0.5)
            m_ref[...] = jnp.full(m_ref.shape, -jnp.inf, jnp.float32)
            l_ref[...] = jnp.zeros(l_ref.shape, jnp.float32)
            acc_ref[...] = jnp.zeros(acc_ref.shape, jnp.float32)

        def o_proj(x):
            out = x
            for g in range(hkv):
                lsum = jnp.sum(l_ref[g], axis=-1, keepdims=True)
                og = (acc_ref[g] / lsum).astype(jnp.bfloat16)
                flat = jnp.concatenate(
                    [jnp.broadcast_to(og[hh:hh + 1, :], (8, _DH)) for hh in range(rep)], axis=1)
                out = out + jnp.dot(flat, wo[g * rep * _DH:(g + 1) * rep * _DH, :],
                                    preferred_element_type=jnp.float32)
            return out

        def mlp_up(x):
            xn = _layernorm(x).astype(jnp.bfloat16)
            h = jnp.dot(xn, w1[...], preferred_element_type=jnp.float32) \
                + b1[...].astype(jnp.float32).reshape(1, f_dim)
            sp = jnp.log1p(jnp.exp(-jnp.abs(h))) + jnp.where(h > 0, h, 0.0)
            return (h * jnp.tanh(sp)).astype(jnp.bfloat16)

        def mlp_down(x, act):
            return x + jnp.dot(act, w2[...], preferred_element_type=jnp.float32)

        def split_rows_copy(src, dst, sem, rows, cols=None):
            n = src.shape[0]
            half = n // 2
            if cols is None:
                def b(i, c):
                    for pr in range(2):
                        r = pl.ds(pl.multiple_of(pr * half + i * rows, rows), rows)
                        pltpu.make_async_copy(src.at[r], dst.at[r], sem).start(priority=pr)
                    return c
                lax.fori_loop(0, half // rows, b, 0)
            else:
                ncol = src.shape[1] // cols

                def b(i, c):
                    for pr in range(2):
                        r = pl.ds(pl.multiple_of(pr * half + (i // ncol) * rows, rows), rows)
                        cc = pl.ds(pl.multiple_of((i % ncol) * cols, cols), cols)
                        pltpu.make_async_copy(src.at[r, cc], dst.at[r, cc], sem).start(priority=pr)
                    return c
                lax.fori_loop(0, (half // rows) * ncol, b, 0)

        c_x = pltpu.make_async_copy(x_hbm, xs, wsem.at[0])
        c_wq = pltpu.make_async_copy(wq_hbm, wq, wsem.at[1])
        c_wo = pltpu.make_async_copy(wo_hbm, wo, wsem.at[2])
        c_w1 = pltpu.make_async_copy(w1_hbm, w1, wsem.at[3])
        c_b1 = pltpu.make_async_copy(b1_hbm, b1, wsem.at[4])
        c_w2 = pltpu.make_async_copy(w2_hbm, w2, wsem.at[5])

        c_x.start()
        if split_w:
            split_rows_copy(wq_hbm, wq, wsem.at[1], 16, 1024)
        else:
            c_wq.start()
        for u in range(R - 1):
            issue(u, u % R)
        if split_w:
            split_rows_copy(wo_hbm, wo, wsem.at[2], 32)
        else:
            c_wo.start()

        def init_redo(i, c):
            redo_ref[i] = i
            return c
        lax.fori_loop(0, M, init_redo, 0)
        redo_ref[U] = M

        with jax.named_scope('head'):
            c_x.wait()
            c_wq.wait()
            x0 = jnp.broadcast_to(xs[...].astype(jnp.float32), (8, _D))
            q_proj(x0)

        def step1(u):
            slot = u % R

            @pl.when(u + R - 1 < U)
            def _():
                issue(u + R - 1, (u + R - 1) % R)
            wait(slot)
            return slot

        def body1a(u, c):
            process_raw(step1(u), u // uph)
            return c
        with jax.named_scope('p1a'):
            lax.fori_loop(0, M, body1a, 0)

        def body1b(u, c):
            process_encode(step1(u), u // uph, u - M)
            return c
        with jax.named_scope('p1b'):
            lax.fori_loop(M, M + NC, body1b, 0)

        with jax.named_scope('p1c'):
            issue(U - 1, (U - 1) % R)
            c_b1.start()
            if split_w:
                split_rows_copy(w1_hbm, w1, wsem.at[3], 16)
                split_rows_copy(w2_hbm, w2, wsem.at[5], 32)
            else:
                c_w1.start()
                c_w2.start()

            def body1c(u, c):
                wait(u % R)
                process_raw(u % R, u // uph)
                return c
            lax.fori_loop(M + NC, U, body1c, 0)

        with jax.named_scope('sync'):
            c_wo.wait()
            x1 = o_proj(x0)
            c_b1.wait()
            c_w1.wait()
            act = mlp_up(x1)
            c_w2.wait()
            x2 = mlp_down(x1, act)
            q_proj(x2)

        n_redo = redo_ref[U]
        with jax.named_scope('p2pro'):
            for i in range(R):
                u = U - R + i
                process_raw(u % R, u // uph)
                if i < R - 1:
                    issue(redo_ref[i], u % R)

        def body2(j, c_done):
            slot = (U + j) % R

            @pl.when(j + R - 1 < n_redo)
            def _():
                issue(redo_ref[j + R - 1], (U + j + R - 1) % R)
            c_next = jnp.minimum(((j + 1) * NC + lead) // n_redo, NC)

            def inner(c, z):
                @pl.when(ok_ref[c] != 0)
                def _():
                    process_packed(c)
                return z
            lax.fori_loop(c_done, c_next, inner, 0)
            wait(slot)

            process_raw(slot, redo_ref[j] // uph)
            return c_next
        with jax.named_scope('p2'):
            lax.fori_loop(0, n_redo, body2, 0)

        with jax.named_scope('tail'):
            x3 = o_proj(x2)
            act = mlp_up(x3)
            x4 = mlp_down(x3, act)
            out_ref[...] = x4[:1, :].astype(out_ref.dtype)

    return pl.pallas_call(
        kernel,
        out_shape=jax.ShapeDtypeStruct((1, _D), jnp.bfloat16),
        in_specs=[pl.BlockSpec(memory_space=pl.ANY)] * 8,
        out_specs=pl.BlockSpec(memory_space=pltpu.VMEM),
        scratch_shapes=[
            pltpu.VMEM((R, BS, _DH), jnp.bfloat16),
            pltpu.VMEM((R, BS, _DH), jnp.bfloat16),
            pltpu.VMEM((NC, NSM * 64, 128), _I32),
            pltpu.VMEM((NC, NE * 64, 128), _I32),
            pltpu.VMEM((NC, NSM * 64, 128), _I32),
            pltpu.VMEM((NC, NE * 64, 128), _I32),
            pltpu.VMEM((_D, _HQ * _DH), jnp.bfloat16),
            pltpu.VMEM((_HQ * _DH, _D), jnp.bfloat16),
            pltpu.VMEM((_D, f_dim), jnp.bfloat16),
            pltpu.VMEM((f_dim, _D), jnp.bfloat16),
            pltpu.VMEM((f_dim,), jnp.bfloat16),
            pltpu.VMEM((1, _D), jnp.bfloat16),
            pltpu.VMEM((hkv, 8, _DH), jnp.float32),
            pltpu.VMEM((hkv, 8, _DH), jnp.float32),
            pltpu.VMEM((hkv, 8, _DH), jnp.float32),
            pltpu.VMEM((hkv, 8, _DH), jnp.float32),
            pltpu.SMEM((2 * NC,), _I32),
            pltpu.SMEM((NC,), _I32),
            pltpu.SMEM((U + 1,), _I32),
            pltpu.SemaphoreType.DMA((R,)),
            pltpu.SemaphoreType.DMA((R,)),
            pltpu.SemaphoreType.DMA((6,)),
        ],
        compiler_params=pltpu.CompilerParams(vmem_limit_bytes=128 * 1024 * 1024,
                                             disable_bounds_checks=nobounds),
    )


@jax.jit
def pallas_interleave_layers__gqa_block_cached__dense_activation_mish__decode_kernel(
    A_x: jax.Array,
    A_k_cache: jax.Array,
    A_v_cache: jax.Array,
    A_wq: jax.Array,
    A_wo: jax.Array,
    B_x: jax.Array,
    B_w1: jax.Array,
    B_b1: jax.Array,
    B_w2: jax.Array,
):
    del B_x
    _, hkv, sk, dh = A_k_cache.shape
    f_dim = B_w1.shape[1]
    out = build(hkv, sk, f_dim, T=32, R=3, NC=65, pieces=(192,) * 20 + (128,) * 2, force_bad=None, nobounds=False, split_w=True, lead_units=1)(
        A_x.reshape(1, _D),
        A_k_cache.reshape(hkv * sk, dh),
        A_v_cache.reshape(hkv * sk, dh),
        A_wq, A_wo, B_w1, B_b1, B_w2)
    return out.reshape(1, 1, _D)
```

```python
import functools

import jax
import jax.numpy as jnp
import numpy as np
from jax import lax
import jax.experimental.pallas as pl
import jax.experimental.pallas.tpu as pltpu

_D = 512
_HQ = 32
_DH = 128
_EPS = 1e-5
_NT = (((1,), (1,)), ((), ()))
_I32 = jnp.int32
_G = 16


def _c32(x):
    return np.int32(np.uint32(x))


def _srl(x, n):
    return lax.shift_right_logical(x, np.int32(n))


def _layernorm(x):
    m = jnp.mean(x, axis=-1, keepdims=True)
    c = x - m
    v = jnp.mean(c * c, axis=-1, keepdims=True)
    return c / jnp.sqrt(v + _EPS)


def build(hkv, sk, f_dim, T, R, NC, pieces, force_bad=None, nobounds=False, slack=3, nsub=4, pack_unroll=4):
    BS = T * 128
    HB = BS // 2
    rep = _HQ // hkv
    GW = rep * _DH
    uph = sk // BS
    U = hkv * uph
    M = U - R - NC
    X = M - 1
    assert T == 2 * _G and sum(pieces) == BS and X >= R and 1 <= slack < X
    lo_tiles = tuple(range(_G))
    hi_tiles = tuple(range(_G, T))
    all_tiles = tuple(range(T))

    def kernel(x_hbm, k_hbm, v_hbm, wq_hbm, wo_hbm, w1_hbm, b1_hbm, w2_hbm, out_ref,
               kbuf, vbuf, ksm, kex, vsm, vex, ksm_h, kex_h, vsm_h, vex_h,
               wq, wo, w1, w2, b1, xs,
               q_ref, m_ref, l_ref, acc_ref, s_ref, base_ref, bad_ref, ok_ref, redo_ref,
               ksem, vsem, wsem):

        def issue_rows(unit, slot, lo, sizes):
            base = pl.multiple_of(unit * BS, BS)
            for n in sizes:
                rows = pl.ds(base + lo, n)
                dst = pl.ds(lo, n)
                pltpu.make_async_copy(k_hbm.at[rows], kbuf.at[slot, dst], ksem.at[slot]).start(priority=0)
                pltpu.make_async_copy(v_hbm.at[rows], vbuf.at[slot, dst], vsem.at[slot]).start(priority=1)
                lo += n

        def issue(unit, slot):
            issue_rows(unit, slot, 0, pieces)

        def issue_k_first(unit, slot, nrows):
            base = pl.multiple_of(unit * BS, BS)
            for src, buf, sem in ((k_hbm, kbuf, ksem), (v_hbm, vbuf, vsem)):
                for off in range(0, nrows // 2, 128):
                    for pr in range(2):
                        o = off + pr * (nrows // 2)
                        pltpu.make_async_copy(src.at[pl.ds(base + o, 128)], buf.at[slot, pl.ds(o, 128)],
                                              sem.at[slot]).start(priority=pr)

        def wait_k(slot, n=BS):
            pltpu.make_async_copy(k_hbm.at[pl.ds(0, n)], kbuf.at[slot, pl.ds(0, n)], ksem.at[slot]).wait()

        def wait_v(slot, n=BS):
            pltpu.make_async_copy(v_hbm.at[pl.ds(0, n)], vbuf.at[slot, pl.ds(0, n)], vsem.at[slot]).wait()

        def wait(slot, n=BS):
            wait_k(slot, n)
            wait_v(slot, n)

        def attend(g, get_k, get_v, tiles=all_tiles, mid=None):
            q = q_ref[g].astype(jnp.bfloat16)
            mxv = None
            for i, t in enumerate(tiles):
                s = lax.dot_general(q, get_k(t), _NT, preferred_element_type=jnp.float32)
                s_ref[i] = s
                mxv = s if mxv is None else jnp.maximum(mxv, s)
            mx = jnp.max(mxv, axis=-1, keepdims=True)
            m_old = m_ref[g]
            m_new = jnp.maximum(m_old, mx)
            alpha = jnp.exp(m_old - m_new)
            m_ref[g] = m_new
            lsum = alpha * l_ref[g]
            acc = alpha * acc_ref[g]
            if mid is not None:
                mid()
            for i, t in enumerate(tiles):
                p = jnp.exp(s_ref[i] - m_new)
                lsum = lsum + p
                acc = acc + jnp.dot(p.astype(jnp.bfloat16), get_v(t),
                                    preferred_element_type=jnp.float32)
            l_ref[g] = lsum
            acc_ref[g] = acc

        def raw_tile(buf, slot):
            return lambda t: buf[slot, t * 128:(t + 1) * 128, :]

        def process_raw(slot, g, tiles=all_tiles, mid=None):
            attend(g, raw_tile(kbuf, slot), raw_tile(vbuf, slot), tiles, mid)

        def pick_base(buf, slot, bidx, t0):
            amax = jnp.max(jnp.abs(buf[slot, t0 * 128:(t0 + 1) * 128, :].astype(jnp.float32)),
                           axis=(0, 1), keepdims=True)
            emax = _srl(pltpu.bitcast(jnp.broadcast_to(amax, (8, 128)), _I32), 23) & 0xFF
            base = jnp.clip(emax - 29, 0, 224)
            basep = (base << 7) | (base << 23)
            base_ref[pl.ds(bidx, 1), :] = basep[:1, :]
            return basep

        def pack_rows(buf, slot, sm_ref, ex_ref, c, t0, grp, i, basep, bad):
            r8 = pl.multiple_of(i * 8, 8)
            ws, ds = [], []
            for tt in range(_G):
                row = pl.multiple_of((t0 + grp * _G + tt) * 128 + i * 16, 16)
                w = pltpu.bitcast(buf[slot, pl.ds(row, 16), :], _I32)
                d = (w & _c32(0x7F807F80)) - basep
                bad = bad | d
                ws.append(w)
                ds.append(d)
                if tt % 2 == 1:
                    w0 = ws[tt - 1]
                    sm_ref[c, pl.ds((grp * 8 + tt // 2) * 64 + r8, 8), :] = (
                        (w0 & _c32(0x007F007F)) | (_srl(w0, 8) & _c32(0x00800080))
                        | ((w & _c32(0x007F007F)) << 8) | (w & _c32(0x80008000)))
            for k in range(5):
                ex_ref[c, pl.ds((grp * 5 + k) * 64 + r8, 8), :] = (
                    _srl(ds[3 * k], 7) | _srl(ds[3 * k + 1], 2) | (ds[3 * k + 2] << 3)
                    | ((ds[_G - 1] << (8 - k)) & _c32(0x80008000)))
            return bad

        def process_encode(slot, g, c, half=False):
            t0 = _G if half else 0
            idx = NC if half else c
            planes = ((kbuf, ksm_h if half else ksm, kex_h if half else kex),
                      (vbuf, vsm_h if half else vsm, vex_h if half else vex))
            bases = [pick_base(planes[a][0], slot, 2 * idx + a, t0) for a in range(2)]
            process_raw(slot, g)

            def pack(i, bad):
                for a in range(2):
                    for grp in range(1 if half else T // _G):
                        bad = pack_rows(planes[a][0], slot, planes[a][1], planes[a][2], c, t0, grp, i,
                                        bases[a], bad)
                return bad
            bad = lax.fori_loop(0, 8, pack, jnp.zeros((8, 128), _I32), unroll=pack_unroll) & _c32(0xF000F000)
            bad_ref[pl.ds(idx, 1), :] = functools.reduce(
                jnp.bitwise_or, [bad[r:r + 1, :] for r in range(8)])

        def collect_flags():
            anybad = jnp.max(jnp.where(bad_ref[...] != 0, 1.0, 0.0)) != 0.0
            if force_bad is not None:
                anybad = True
            redo_ref[U] = X

            @pl.when(anybad)
            def _():
                def b(idx, n):
                    ok = jnp.max(jnp.where(bad_ref[pl.ds(idx, 1), :] != 0, 1.0, 0.0)) == 0.0
                    if force_bad is not None:
                        ok = jnp.logical_and(ok, (idx % force_bad) != 2)
                    ok_ref[idx] = ok.astype(_I32)
                    redo_ref[n] = M + idx
                    return n + jnp.where(jnp.logical_or(ok, idx == NC), 0, 1)
                redo_ref[U] = lax.fori_loop(0, NC + 1, b, X)
            return redo_ref[U]

        def decoder(sm_ref, ex_ref, c, bidx, t0):
            basep = jnp.broadcast_to(base_ref[pl.ds(bidx, 1), :], (64, 128))

            def get(t):
                s0 = ((t - t0) // 2) * 64
                sm = sm_ref[c, s0:s0 + 64, :]
                grp, tt = divmod(t - t0, _G)
                if tt < _G - 1:
                    k, j = divmod(tt, 3)
                    e0 = (grp * 5 + k) * 64
                    e = ex_ref[c, e0:e0 + 64, :]
                    e = (e << 7) if j == 0 else (e << 2) if j == 1 else _srl(e, 3)
                    ef = e & _c32(0x0F800F80)
                else:
                    ef = None
                    for k in range(5):
                        e0 = (grp * 5 + k) * 64
                        bit = _srl(ex_ref[c, e0:e0 + 64, :], 8 - k) & _c32(0x00800080 << k)
                        ef = bit if ef is None else ef | bit
                if tt % 2 == 0:
                    a = sm & _c32(0x00FF00FF)
                    a = (a | (a << 8)) & _c32(0x807F807F)
                else:
                    a = sm & _c32(0xFF00FF00)
                    a = (a | _srl(a, 8)) & _c32(0x807F807F)
                return pltpu.bitcast((a | ef) + basep, jnp.bfloat16)
            return get

        def process_packed(c):
            attend((M + c) // uph, decoder(ksm, kex, c, 2 * c, 0), decoder(vsm, vex, c, 2 * c + 1, 0))

        row128 = lax.broadcasted_iota(_I32, (8, _DH), 0)

        def q_proj(xn, heads):
            for g in heads:
                qf = jnp.dot(xn, wq[:, g * GW:(g + 1) * GW], preferred_element_type=jnp.float32)
                qg = jnp.zeros((8, _DH), jnp.float32)
                for hh in range(rep):
                    qg = jnp.where(row128 == hh, qf[:, hh * _DH:(hh + 1) * _DH], qg)
                q_ref[g] = qg * (_DH ** -0.5)

        def reset():
            m_ref[...] = jnp.full(m_ref.shape, -jnp.inf, jnp.float32)
            l_ref[...] = jnp.zeros(l_ref.shape, jnp.float32)
            acc_ref[...] = jnp.zeros(acc_ref.shape, jnp.float32)

        def o_proj(x, heads):
            for g in heads:
                lsum = jnp.sum(l_ref[g], axis=-1, keepdims=True)
                og = (acc_ref[g] / lsum).astype(jnp.bfloat16)
                flat = jnp.concatenate(
                    [jnp.broadcast_to(og[hh:hh + 1, :], (8, _DH)) for hh in range(rep)], axis=1)
                x = x + jnp.dot(flat, wo[g * GW:(g + 1) * GW, :], preferred_element_type=jnp.float32)
            return x

        def mlp_up(x):
            xn = _layernorm(x).astype(jnp.bfloat16)
            h = jnp.dot(xn, w1[...], preferred_element_type=jnp.float32) \
                + b1[...].astype(jnp.float32).reshape(1, f_dim)
            sp = jnp.log1p(jnp.exp(-jnp.abs(h))) + jnp.where(h > 0, h, 0.0)
            return (h * jnp.tanh(sp)).astype(jnp.bfloat16)

        def mlp_down(x, act):
            return x + jnp.dot(act, w2[...], preferred_element_type=jnp.float32)

        def start_weight(src, dst, sem, rows, cols=None):
            half = src.shape[0] // 2
            ncol = 1 if cols is None else src.shape[1] // cols

            def b(i, c):
                for pr in range(2):
                    r = pl.ds(pl.multiple_of(pr * half + (i // ncol) * rows, rows), rows)
                    if cols is None:
                        pltpu.make_async_copy(src.at[r], dst.at[r], sem).start(priority=pr)
                    else:
                        cc = pl.ds(pl.multiple_of((i % ncol) * cols, cols), cols)
                        pltpu.make_async_copy(src.at[r, cc], dst.at[r, cc], sem).start(priority=pr)
                return c
            lax.fori_loop(0, (half // rows) * ncol, b, 0)

        c_x = pltpu.make_async_copy(x_hbm, xs, wsem.at[0])
        c_wq = pltpu.make_async_copy(wq_hbm, wq, wsem.at[1])
        c_wo = pltpu.make_async_copy(wo_hbm, wo, wsem.at[2])
        c_w1 = pltpu.make_async_copy(w1_hbm, w1, wsem.at[3])
        c_b1 = pltpu.make_async_copy(b1_hbm, b1, wsem.at[4])
        c_w2 = pltpu.make_async_copy(w2_hbm, w2, wsem.at[5])

        c_x.start()
        start_weight(wq_hbm, wq, wsem.at[1], 16, 1024)
        for u in range(R - 1):
            issue(u, u % R)
        start_weight(wo_hbm, wo, wsem.at[2], 32)

        def init_redo(i, c):
            redo_ref[i] = i
            return c
        lax.fori_loop(0, X, init_redo, 0)

        def init_ok(i, c):
            ok_ref[i] = 1
            return c
        lax.fori_loop(0, NC + 1, init_ok, 0)

        c_x.wait()
        c_wq.wait()
        x0 = jnp.broadcast_to(xs[...].astype(jnp.float32), (8, _D))
        q_proj(_layernorm(x0).astype(jnp.bfloat16), range(hkv))
        reset()

        def step1(u):
            issue(u + R - 1, (u + R - 1) % R)
            wait(u % R)
            return u % R

        def body1a(u, c):
            process_raw(step1(u), u // uph)
            return c
        lax.fori_loop(0, X, body1a, 0)

        process_encode(step1(X), X // uph, 0, half=True)

        def body1b(u, c):
            process_encode(step1(u), u // uph, u - M)
            return c
        lax.fori_loop(M, M + NC, body1b, 0)

        issue(U - 1, (U - 1) % R)
        c_b1.start()
        start_weight(w1_hbm, w1, wsem.at[3], 16)
        start_weight(w2_hbm, w2, wsem.at[5], 32)
        n_redo = collect_flags()

        def body1c(u, c):
            wait(u % R)
            process_raw(u % R, u // uph)
            return c
        lax.fori_loop(M + NC, U, body1c, 0)

        c_wo.wait()
        x1 = o_proj(x0, range(hkv))
        c_b1.wait()
        c_w1.wait()
        act = mlp_up(x1)
        c_w2.wait()
        x2 = mlp_down(x1, act)
        xn2 = _layernorm(x2).astype(jnp.bfloat16)
        q_proj(xn2, [hkv - 1])
        reset()

        step = T // nsub
        u = U - R
        for sub in range(nsub):
            process_raw(u % R, u // uph, tiles=tuple(range(sub * step, (sub + 1) * step)))
            issue_rows(redo_ref[0], u % R, sub * step * 128, (128,) * step)
        for i in range(1, R):
            u = U - R + i
            process_raw(u % R, u // uph)
            if i < R - 1:
                issue(redo_ref[i], u % R)
            if i == 1:
                q_proj(xn2, range(hkv - 1))

        @pl.when(ok_ref[NC] != 0)
        def _():
            attend(X // uph, decoder(ksm_h, kex_h, 0, 2 * NC, _G),
                   decoder(vsm_h, vex_h, 0, 2 * NC + 1, _G), tiles=hi_tiles)

        def body2(j, c_done):
            slot = (U + j) % R

            @pl.when(j + R - 1 < n_redo)
            def _():
                issue(redo_ref[j + R - 1], (U + j + R - 1) % R)

            @pl.when(j + R - 1 == n_redo)
            def _():
                issue_k_first(X, (U + n_redo) % R, HB)

            c_next = jnp.minimum(((j + 1) * NC) // (n_redo - slack), NC)

            def inner(c, z):
                @pl.when(ok_ref[c] != 0)
                def _():
                    process_packed(c)
                return z
            lax.fori_loop(c_done, c_next, inner, 0)
            wait(slot)
            process_raw(slot, redo_ref[j] // uph)
            return c_next
        lax.fori_loop(0, n_redo, body2, 0)

        @pl.when(ok_ref[NC] == 0)
        def _():
            slot = (U + n_redo - 1) % R
            issue_rows(X, slot, HB, (128,) * _G)
            wait(slot, HB)
            process_raw(slot, X // uph, tiles=hi_tiles)

        g_last = X // uph
        slot = (U + n_redo) % R
        x3 = o_proj(x2, [g for g in range(hkv) if g != g_last])
        wait_k(slot, HB)
        process_raw(slot, g_last, tiles=lo_tiles, mid=lambda: wait_v(slot, HB))
        x3 = o_proj(x3, [g_last])
        x4 = mlp_down(x3, mlp_up(x3))
        out_ref[...] = x4[:1, :].astype(out_ref.dtype)

    nsm, nex = T // 2 * 64, T // _G * 5 * 64
    return pl.pallas_call(
        kernel,
        out_shape=jax.ShapeDtypeStruct((1, _D), jnp.bfloat16),
        in_specs=[pl.BlockSpec(memory_space=pl.ANY)] * 8,
        out_specs=pl.BlockSpec(memory_space=pltpu.VMEM),
        scratch_shapes=[
            pltpu.VMEM((R, BS, _DH), jnp.bfloat16),
            pltpu.VMEM((R, BS, _DH), jnp.bfloat16),
            pltpu.VMEM((NC, nsm, 128), _I32),
            pltpu.VMEM((NC, nex, 128), _I32),
            pltpu.VMEM((NC, nsm, 128), _I32),
            pltpu.VMEM((NC, nex, 128), _I32),
            pltpu.VMEM((1, nsm // 2, 128), _I32),
            pltpu.VMEM((1, nex // 2, 128), _I32),
            pltpu.VMEM((1, nsm // 2, 128), _I32),
            pltpu.VMEM((1, nex // 2, 128), _I32),
            pltpu.VMEM((_D, _HQ * _DH), jnp.bfloat16),
            pltpu.VMEM((_HQ * _DH, _D), jnp.bfloat16),
            pltpu.VMEM((_D, f_dim), jnp.bfloat16),
            pltpu.VMEM((f_dim, _D), jnp.bfloat16),
            pltpu.VMEM((f_dim,), jnp.bfloat16),
            pltpu.VMEM((1, _D), jnp.bfloat16),
            pltpu.VMEM((hkv, 8, _DH), jnp.float32),
            pltpu.VMEM((hkv, 8, _DH), jnp.float32),
            pltpu.VMEM((hkv, 8, _DH), jnp.float32),
            pltpu.VMEM((hkv, 8, _DH), jnp.float32),
            pltpu.VMEM((T, 8, _DH), jnp.float32),
            pltpu.VMEM((2 * NC + 2, 128), _I32),
            pltpu.VMEM((NC + 1, 128), _I32),
            pltpu.SMEM((NC + 1,), _I32),
            pltpu.SMEM((U + 1,), _I32),
            pltpu.SemaphoreType.DMA((R,)),
            pltpu.SemaphoreType.DMA((R,)),
            pltpu.SemaphoreType.DMA((6,)),
        ],
        compiler_params=pltpu.CompilerParams(vmem_limit_bytes=128 * 1024 * 1024,
                                             disable_bounds_checks=nobounds),
    )


@jax.jit
def pallas_interleave_layers__gqa_block_cached__dense_activation_mish__decode_kernel(
    A_x: jax.Array,
    A_k_cache: jax.Array,
    A_v_cache: jax.Array,
    A_wq: jax.Array,
    A_wo: jax.Array,
    B_x: jax.Array,
    B_w1: jax.Array,
    B_b1: jax.Array,
    B_w2: jax.Array,
):
    del B_x
    _, hkv, sk, dh = A_k_cache.shape
    f_dim = B_w1.shape[1]
    out = build(hkv, sk, f_dim, T=32, R=3, NC=67, pieces=(192,) * 20 + (128,) * 2, force_bad=None, nobounds=False, slack=3, nsub=4, pack_unroll=4)(
        A_x.reshape(1, _D),
        A_k_cache.reshape(hkv * sk, dh),
        A_v_cache.reshape(hkv * sk, dh),
        A_wq, A_wo, B_w1, B_b1, B_w2)
    return out.reshape(1, 1, _D)
```

```python
import functools

import jax
import jax.numpy as jnp
import numpy as np
from jax import lax
import jax.experimental.pallas as pl
import jax.experimental.pallas.tpu as pltpu

_D = 512
_HQ = 32
_DH = 128
_EPS = 1e-5
_NT = (((1,), (1,)), ((), ()))
_I32 = jnp.int32
_G = 16


def _c32(x):
    return np.int32(np.uint32(x))


def _srl(x, n):
    return lax.shift_right_logical(x, np.int32(n))


def _layernorm(x):
    m = jnp.mean(x, axis=-1, keepdims=True)
    c = x - m
    v = jnp.mean(c * c, axis=-1, keepdims=True)
    return c / jnp.sqrt(v + _EPS)


def build(hkv, sk, f_dim, T, R, NC, pieces, slack=3, nsub=4, pack_unroll=4):
    BS = T * 128
    HB = BS // 2
    rep = _HQ // hkv
    GW = rep * _DH
    uph = sk // BS
    U = hkv * uph
    M = U - R - NC
    X = M - 1
    assert T == 2 * _G and sum(pieces) == BS and X >= R and 1 <= slack < X
    lo_tiles = tuple(range(_G))
    hi_tiles = tuple(range(_G, T))
    all_tiles = tuple(range(T))

    def kernel(x_hbm, k_hbm, v_hbm, wq_hbm, wo_hbm, w1_hbm, b1_hbm, w2_hbm, out_ref,
               kbuf, vbuf, ksm, kex, vsm, vex, ksm_h, kex_h, vsm_h, vex_h,
               wq, wo, w1, w2, b1, xs,
               q_ref, m_ref, l_ref, acc_ref, s_ref, base_ref, bad_ref, ok_ref, redo_ref,
               ksem, vsem, wsem):

        def issue_rows(unit, slot, lo, sizes):
            base = pl.multiple_of(unit * BS, BS)
            for n in sizes:
                rows = pl.ds(base + lo, n)
                dst = pl.ds(lo, n)
                pltpu.make_async_copy(k_hbm.at[rows], kbuf.at[slot, dst], ksem.at[slot]).start(priority=0)
                pltpu.make_async_copy(v_hbm.at[rows], vbuf.at[slot, dst], vsem.at[slot]).start(priority=1)
                lo += n

        def issue(unit, slot):
            issue_rows(unit, slot, 0, pieces)

        def issue_k_first(unit, slot, nrows):
            base = pl.multiple_of(unit * BS, BS)
            for src, buf, sem in ((k_hbm, kbuf, ksem), (v_hbm, vbuf, vsem)):
                for off in range(0, nrows // 2, 128):
                    for pr in range(2):
                        o = off + pr * (nrows // 2)
                        pltpu.make_async_copy(src.at[pl.ds(base + o, 128)], buf.at[slot, pl.ds(o, 128)],
                                              sem.at[slot]).start(priority=pr)

        def wait_k(slot, n=BS, lo=0):
            pltpu.make_async_copy(k_hbm.at[pl.ds(lo, n)], kbuf.at[slot, pl.ds(lo, n)], ksem.at[slot]).wait()

        def wait_v(slot, n=BS, lo=0):
            pltpu.make_async_copy(v_hbm.at[pl.ds(lo, n)], vbuf.at[slot, pl.ds(lo, n)], vsem.at[slot]).wait()

        def wait(slot, n=BS, lo=0):
            wait_k(slot, n, lo)
            wait_v(slot, n, lo)

        def attend(g, get_k, get_v, tiles=all_tiles, mid=None):
            q = q_ref[g].astype(jnp.bfloat16)
            mxv = None
            for i, t in enumerate(tiles):
                s = lax.dot_general(q, get_k(t), _NT, preferred_element_type=jnp.float32)
                s_ref[i] = s
                mxv = s if mxv is None else jnp.maximum(mxv, s)
            mx = jnp.max(mxv, axis=-1, keepdims=True)
            m_old = m_ref[g]
            m_new = jnp.maximum(m_old, mx)
            alpha = jnp.exp(m_old - m_new)
            m_ref[g] = m_new
            lsum = alpha * l_ref[g]
            acc = alpha * acc_ref[g]
            if mid is not None:
                mid()
            for i, t in enumerate(tiles):
                p = jnp.exp(s_ref[i] - m_new)
                lsum = lsum + p
                acc = acc + jnp.dot(p.astype(jnp.bfloat16), get_v(t),
                                    preferred_element_type=jnp.float32)
            l_ref[g] = lsum
            acc_ref[g] = acc

        def raw_tile(buf, slot):
            return lambda t: buf[slot, t * 128:(t + 1) * 128, :]

        def process_raw(slot, g, tiles=all_tiles, mid=None):
            attend(g, raw_tile(kbuf, slot), raw_tile(vbuf, slot), tiles, mid)

        def pick_base(buf, slot, bidx, t0):
            amax = jnp.max(jnp.abs(buf[slot, t0 * 128:(t0 + 1) * 128, :].astype(jnp.float32)),
                           axis=(0, 1), keepdims=True)
            emax = _srl(pltpu.bitcast(jnp.broadcast_to(amax, (8, 128)), _I32), 23) & 0xFF
            base = jnp.clip(emax - 29, 0, 224)
            basep = (base << 7) | (base << 23)
            base_ref[pl.ds(bidx, 1), :] = basep[:1, :]
            return basep

        def pack_rows(buf, slot, sm_ref, ex_ref, c, t0, grp, i, basep, bad):
            r8 = pl.multiple_of(i * 8, 8)
            ws, ds = [], []
            for tt in range(_G):
                row = pl.multiple_of((t0 + grp * _G + tt) * 128 + i * 16, 16)
                w = pltpu.bitcast(buf[slot, pl.ds(row, 16), :], _I32)
                d = (w & _c32(0x7F807F80)) - basep
                bad = bad | d
                ws.append(w)
                ds.append(d)
                if tt % 2 == 1:
                    w0 = ws[tt - 1]
                    sm_ref[c, pl.ds((grp * 8 + tt // 2) * 64 + r8, 8), :] = (
                        (w0 & _c32(0x007F007F)) | (_srl(w0, 8) & _c32(0x00800080))
                        | ((w & _c32(0x007F007F)) << 8) | (w & _c32(0x80008000)))
            for k in range(5):
                ex_ref[c, pl.ds((grp * 5 + k) * 64 + r8, 8), :] = (
                    _srl(ds[3 * k], 7) | _srl(ds[3 * k + 1], 2) | (ds[3 * k + 2] << 3)
                    | ((ds[_G - 1] << (8 - k)) & _c32(0x80008000)))
            return bad

        def process_encode(slot, g, c, half=False):
            t0 = _G if half else 0
            idx = NC if half else c
            planes = ((kbuf, ksm_h if half else ksm, kex_h if half else kex),
                      (vbuf, vsm_h if half else vsm, vex_h if half else vex))
            bases = [pick_base(planes[a][0], slot, 2 * idx + a, t0) for a in range(2)]
            process_raw(slot, g)

            def pack(i, bad):
                for a in range(2):
                    for grp in range(1 if half else T // _G):
                        bad = pack_rows(planes[a][0], slot, planes[a][1], planes[a][2], c, t0, grp, i,
                                        bases[a], bad)
                return bad
            bad = lax.fori_loop(0, 8, pack, jnp.zeros((8, 128), _I32), unroll=pack_unroll) & _c32(0xF000F000)
            bad_ref[pl.ds(idx, 1), :] = functools.reduce(
                jnp.bitwise_or, [bad[r:r + 1, :] for r in range(8)])

        def collect_flags():
            anybad = jnp.max(jnp.where(bad_ref[...] != 0, 1.0, 0.0)) != 0.0
            redo_ref[U] = X

            @pl.when(anybad)
            def _():
                def b(idx, n):
                    ok = jnp.max(jnp.where(bad_ref[pl.ds(idx, 1), :] != 0, 1.0, 0.0)) == 0.0
                    ok_ref[idx] = ok.astype(_I32)
                    redo_ref[n] = M + idx
                    return n + jnp.where(jnp.logical_or(ok, idx == NC), 0, 1)
                redo_ref[U] = lax.fori_loop(0, NC + 1, b, X)
            return redo_ref[U]

        def decoder(sm_ref, ex_ref, c, bidx, t0):
            basep = jnp.broadcast_to(base_ref[pl.ds(bidx, 1), :], (64, 128))

            def get(t):
                s0 = ((t - t0) // 2) * 64
                sm = sm_ref[c, s0:s0 + 64, :]
                grp, tt = divmod(t - t0, _G)
                if tt < _G - 1:
                    k, j = divmod(tt, 3)
                    e0 = (grp * 5 + k) * 64
                    e = ex_ref[c, e0:e0 + 64, :]
                    e = (e << 7) if j == 0 else (e << 2) if j == 1 else _srl(e, 3)
                    ef = e & _c32(0x0F800F80)
                else:
                    ef = None
                    for k in range(5):
                        e0 = (grp * 5 + k) * 64
                        bit = _srl(ex_ref[c, e0:e0 + 64, :], 8 - k) & _c32(0x00800080 << k)
                        ef = bit if ef is None else ef | bit
                if tt % 2 == 0:
                    a = sm & _c32(0x00FF00FF)
                    a = (a | (a << 8)) & _c32(0x807F807F)
                else:
                    a = sm & _c32(0xFF00FF00)
                    a = (a | _srl(a, 8)) & _c32(0x807F807F)
                return pltpu.bitcast((a | ef) + basep, jnp.bfloat16)
            return get

        def process_packed(c):
            attend((M + c) // uph, decoder(ksm, kex, c, 2 * c, 0), decoder(vsm, vex, c, 2 * c + 1, 0))

        row128 = lax.broadcasted_iota(_I32, (8, _DH), 0)

        def q_proj(xn, heads):
            for g in heads:
                qf = jnp.dot(xn, wq[:, g * GW:(g + 1) * GW], preferred_element_type=jnp.float32)
                qg = jnp.zeros((8, _DH), jnp.float32)
                for hh in range(rep):
                    qg = jnp.where(row128 == hh, qf[:, hh * _DH:(hh + 1) * _DH], qg)
                q_ref[g] = qg * (_DH ** -0.5)

        def reset():
            m_ref[...] = jnp.full(m_ref.shape, -jnp.inf, jnp.float32)
            l_ref[...] = jnp.zeros(l_ref.shape, jnp.float32)
            acc_ref[...] = jnp.zeros(acc_ref.shape, jnp.float32)

        def o_proj(x, heads):
            for g in heads:
                lsum = jnp.sum(l_ref[g], axis=-1, keepdims=True)
                og = (acc_ref[g] / lsum).astype(jnp.bfloat16)
                flat = jnp.concatenate(
                    [jnp.broadcast_to(og[hh:hh + 1, :], (8, _DH)) for hh in range(rep)], axis=1)
                x = x + jnp.dot(flat, wo[g * GW:(g + 1) * GW, :], preferred_element_type=jnp.float32)
            return x

        def mlp_up(x):
            xn = _layernorm(x).astype(jnp.bfloat16)
            h = jnp.dot(xn, w1[...], preferred_element_type=jnp.float32) \
                + b1[...].astype(jnp.float32).reshape(1, f_dim)
            sp = jnp.log1p(jnp.exp(-jnp.abs(h))) + jnp.where(h > 0, h, 0.0)
            return (h * jnp.tanh(sp)).astype(jnp.bfloat16)

        def mlp_down(x, act):
            return x + jnp.dot(act, w2[...], preferred_element_type=jnp.float32)

        def start_weight(src, dst, sem, rows, cols=None):
            half = src.shape[0] // 2
            ncol = 1 if cols is None else src.shape[1] // cols

            def b(i, c):
                for pr in range(2):
                    r = pl.ds(pl.multiple_of(pr * half + (i // ncol) * rows, rows), rows)
                    if cols is None:
                        pltpu.make_async_copy(src.at[r], dst.at[r], sem).start(priority=pr)
                    else:
                        cc = pl.ds(pl.multiple_of((i % ncol) * cols, cols), cols)
                        pltpu.make_async_copy(src.at[r, cc], dst.at[r, cc], sem).start(priority=pr)
                return c
            lax.fori_loop(0, (half // rows) * ncol, b, 0)

        c_x = pltpu.make_async_copy(x_hbm, xs, wsem.at[0])
        c_wq = pltpu.make_async_copy(wq_hbm, wq, wsem.at[1])
        c_wo = pltpu.make_async_copy(wo_hbm, wo, wsem.at[2])
        c_w1 = pltpu.make_async_copy(w1_hbm, w1, wsem.at[3])
        c_b1 = pltpu.make_async_copy(b1_hbm, b1, wsem.at[4])
        c_w2 = pltpu.make_async_copy(w2_hbm, w2, wsem.at[5])

        c_x.start()
        start_weight(wq_hbm, wq, wsem.at[1], 16, 1024)
        for u in range(R - 1):
            issue(u, u % R)
        start_weight(wo_hbm, wo, wsem.at[2], 32)

        def init_redo(i, c):
            redo_ref[i] = i
            return c
        lax.fori_loop(0, X, init_redo, 0)

        def init_ok(i, c):
            ok_ref[i] = 1
            return c
        lax.fori_loop(0, NC + 1, init_ok, 0)

        c_x.wait()
        c_wq.wait()
        x0 = jnp.broadcast_to(xs[...].astype(jnp.float32), (8, _D))
        q_proj(_layernorm(x0).astype(jnp.bfloat16), range(hkv))
        reset()

        def step1(u):
            issue(u + R - 1, (u + R - 1) % R)
            wait(u % R)
            return u % R

        def body1a(u, c):
            process_raw(step1(u), u // uph)
            return c
        lax.fori_loop(0, X, body1a, 0)

        process_encode(step1(X), X // uph, 0, half=True)

        def body1b(u, c):
            process_encode(step1(u), u // uph, u - M)
            return c
        lax.fori_loop(M, M + NC, body1b, 0)

        issue(U - 1, (U - 1) % R)
        c_b1.start()
        start_weight(w1_hbm, w1, wsem.at[3], 16)
        start_weight(w2_hbm, w2, wsem.at[5], 32)
        n_redo = collect_flags()

        def body1c(u, c):
            wait(u % R)
            process_raw(u % R, u // uph)
            return c
        lax.fori_loop(M + NC, U, body1c, 0)

        c_wo.wait()
        x1 = o_proj(x0, range(hkv))
        c_b1.wait()
        c_w1.wait()
        act = mlp_up(x1)
        c_w2.wait()
        x2 = mlp_down(x1, act)
        xn2 = _layernorm(x2).astype(jnp.bfloat16)
        q_proj(xn2, [hkv - 1])
        reset()

        step = T // nsub
        u = U - R
        for sub in range(nsub):
            process_raw(u % R, u // uph, tiles=tuple(range(sub * step, (sub + 1) * step)))
            issue_rows(redo_ref[0], u % R, sub * step * 128, (128,) * step)
        for i in range(1, R):
            u = U - R + i
            process_raw(u % R, u // uph)
            if i < R - 1:
                issue(redo_ref[i], u % R)
            if i == 1:
                q_proj(xn2, range(hkv - 1))

        @pl.when(ok_ref[NC] != 0)
        def _():
            attend(X // uph, decoder(ksm_h, kex_h, 0, 2 * NC, _G),
                   decoder(vsm_h, vex_h, 0, 2 * NC + 1, _G), tiles=hi_tiles)

        def body2(j, c_done):
            slot = (U + j) % R

            @pl.when(j + R - 1 < n_redo)
            def _():
                issue(redo_ref[j + R - 1], (U + j + R - 1) % R)

            @pl.when(j + R - 1 == n_redo)
            def _():
                issue_k_first(X, (U + n_redo) % R, HB)

            c_next = jnp.minimum(((j + 1) * NC) // (n_redo - slack), NC)

            def inner(c, z):
                @pl.when(ok_ref[c] != 0)
                def _():
                    process_packed(c)
                return z
            lax.fori_loop(c_done, c_next, inner, 0)
            wait(slot)
            process_raw(slot, redo_ref[j] // uph)
            return c_next
        lax.fori_loop(0, n_redo, body2, 0)

        @pl.when(ok_ref[NC] == 0)
        def _():
            slot = (U + n_redo - 1) % R
            issue_rows(X, slot, HB, (128,) * _G)
            wait(slot, HB, HB)
            process_raw(slot, X // uph, tiles=hi_tiles)

        g_last = X // uph
        slot = (U + n_redo) % R
        x3 = o_proj(x2, [g for g in range(hkv) if g != g_last])
        wait_k(slot, HB)
        process_raw(slot, g_last, tiles=lo_tiles, mid=lambda: wait_v(slot, HB))
        x3 = o_proj(x3, [g_last])
        x4 = mlp_down(x3, mlp_up(x3))
        out_ref[...] = x4[:1, :].astype(out_ref.dtype)

    nsm, nex = T // 2 * 64, T // _G * 5 * 64
    return pl.pallas_call(
        kernel,
        out_shape=jax.ShapeDtypeStruct((1, _D), jnp.bfloat16),
        in_specs=[pl.BlockSpec(memory_space=pl.ANY)] * 8,
        out_specs=pl.BlockSpec(memory_space=pltpu.VMEM),
        scratch_shapes=[
            pltpu.VMEM((R, BS, _DH), jnp.bfloat16),
            pltpu.VMEM((R, BS, _DH), jnp.bfloat16),
            pltpu.VMEM((NC, nsm, 128), _I32),
            pltpu.VMEM((NC, nex, 128), _I32),
            pltpu.VMEM((NC, nsm, 128), _I32),
            pltpu.VMEM((NC, nex, 128), _I32),
            pltpu.VMEM((1, nsm // 2, 128), _I32),
            pltpu.VMEM((1, nex // 2, 128), _I32),
            pltpu.VMEM((1, nsm // 2, 128), _I32),
            pltpu.VMEM((1, nex // 2, 128), _I32),
            pltpu.VMEM((_D, _HQ * _DH), jnp.bfloat16),
            pltpu.VMEM((_HQ * _DH, _D), jnp.bfloat16),
            pltpu.VMEM((_D, f_dim), jnp.bfloat16),
            pltpu.VMEM((f_dim, _D), jnp.bfloat16),
            pltpu.VMEM((f_dim,), jnp.bfloat16),
            pltpu.VMEM((1, _D), jnp.bfloat16),
            pltpu.VMEM((hkv, 8, _DH), jnp.float32),
            pltpu.VMEM((hkv, 8, _DH), jnp.float32),
            pltpu.VMEM((hkv, 8, _DH), jnp.float32),
            pltpu.VMEM((hkv, 8, _DH), jnp.float32),
            pltpu.VMEM((T, 8, _DH), jnp.float32),
            pltpu.VMEM((2 * NC + 2, 128), _I32),
            pltpu.VMEM((NC + 1, 128), _I32),
            pltpu.SMEM((NC + 1,), _I32),
            pltpu.SMEM((U + 1,), _I32),
            pltpu.SemaphoreType.DMA((R,)),
            pltpu.SemaphoreType.DMA((R,)),
            pltpu.SemaphoreType.DMA((6,)),
        ],
        compiler_params=pltpu.CompilerParams(vmem_limit_bytes=128 * 1024 * 1024),
    )


@jax.jit
def pallas_interleave_layers__gqa_block_cached__dense_activation_mish__decode_kernel(
    A_x: jax.Array,
    A_k_cache: jax.Array,
    A_v_cache: jax.Array,
    A_wq: jax.Array,
    A_wo: jax.Array,
    B_x: jax.Array,
    B_w1: jax.Array,
    B_b1: jax.Array,
    B_w2: jax.Array,
):
    del B_x
    _, hkv, sk, dh = A_k_cache.shape
    f_dim = B_w1.shape[1]
    out = build(hkv, sk, f_dim, T=32, R=3, NC=67, pieces=(192,) * 20 + (128,) * 2, slack=3, nsub=4, pack_unroll=4)(
        A_x.reshape(1, _D),
        A_k_cache.reshape(hkv * sk, dh),
        A_v_cache.reshape(hkv * sk, dh),
        A_wq, A_wo, B_w1, B_b1, B_w2)
    return out.reshape(1, 1, _D)
```
